```python
import jax
import jax.numpy as jnp

def _softmax(x, axis=-1):
    return jax.nn.softmax(x, axis=axis)
def _gelu(x):
    return jax.nn.gelu(x, approximate=True)
def _silu(x):
    return jax.nn.silu(x)
def _sigmoid(x):
    return jax.nn.sigmoid(x)
def _layernorm(x, axis=-1, eps=1e-5):
    m = jnp.mean(x, axis=axis, keepdims=True)
    v = jnp.var(x, axis=axis, keepdims=True)
    return (x - m) / jnp.sqrt(v + eps)
def _scatter_add(tgt, idx, src, axis=0):
    return tgt.at[idx].add(src)
def _segment_sum(src, seg, n):
    return jax.ops.segment_sum(src, seg, n)
class _Rng:
    def __init__(self, key):
        self._k = key
    def _next(self):
        self._k, sub = jax.random.split(self._k)
        return sub
    def normal(self, shape):
        return jax.random.normal(self._next(), shape, dtype=jnp.bfloat16)
    def randint(self, lo, hi, shape):
        return jax.random.randint(self._next(), shape, lo, hi, dtype=jnp.int32)
    def uniform(self, shape, lo=0.0, hi=1.0):
        return jax.random.uniform(self._next(), shape, jnp.bfloat16, lo, hi)
    def permutation(self, n):
        return jax.random.permutation(self._next(), n)


kernel_name = 'recurrent_scan__compressed_kv_cla__dense_activation_gelu__decode'

def setup_inputs():
    _rng = _Rng(jax.random.key(int.from_bytes(__import__("os").urandom(4), "little")))
    _w = (lambda a: (lambda t: t.astype(jnp.bfloat16) if jnp.issubdtype(t.dtype, jnp.floating) else t)(jnp.asarray(a)))
    def _A_setup():
        B, H, Sq, Sk, D, M = 2, 32, 1, 16384, 128, 512
        Dc = 4 * D
        return {
            "x": _w((lambda *s: _rng.normal(s) * 0.05)(B, Sq, M)),
            "c_kv": _w((lambda *s: _rng.normal(s) * 0.05)(B, Sk, Dc)),
            "w_q": _w((lambda *s: _rng.normal(s) * 0.05)(M, H, D) * (M ** -0.5)),
            "w_uk": _w((lambda *s: _rng.normal(s) * 0.05)(Dc, H, D) * (Dc ** -0.5)),
            "w_uv": _w((lambda *s: _rng.normal(s) * 0.05)(Dc, H, D) * (Dc ** -0.5)),
            "w_o": _w((lambda *s: _rng.normal(s) * 0.05)(H, D, M) * ((H * D) ** -0.5)),
        }
    _A_in = _A_setup()

    def _B_setup():
        B, S, D, F = 2, 1, 512, 1792
        return {
            "x": _w((lambda *s: _rng.normal(s) * 0.05)(B, S, D)),
            "w1": _w((lambda *s: _rng.normal(s) * 0.05)(D, F) * (D ** -0.5)),
            "b1": _w((lambda *s: _rng.normal(s) * 0.05)(F) * 0.01),
            "w2": _w((lambda *s: _rng.normal(s) * 0.05)(F, D) * (F ** -0.5)),
            "b2": _w((lambda *s: _rng.normal(s) * 0.05)(D) * 0.01),
        }
    _B_in = _B_setup()

    return {
        "A_x": _A_in["x"],
        "A_c_kv": _A_in["c_kv"],
        "A_w_q": _A_in["w_q"],
        "A_w_uk": _A_in["w_uk"],
        "A_w_uv": _A_in["w_uv"],
        "A_w_o": _A_in["w_o"],
        "B_x": _B_in["x"],
        "B_w1": _B_in["w1"],
        "B_b1": _B_in["b1"],
        "B_w2": _B_in["w2"],
        "B_b2": _B_in["b2"],
    }

def reference(A_x, A_c_kv, A_w_q, A_w_uk, A_w_uv, A_w_o, B_x, B_w1, B_b1, B_w2, B_b2):
    def _A_ref(x, c_kv, w_q, w_uk, w_uv, w_o):
        B, Sq, M = x.shape[0], x.shape[1], x.shape[2]
        Sk = c_kv.shape[1]
        H, D = w_q.shape[1], w_q.shape[2]
        q = jnp.einsum("bqm,mhd->bhqd", x, w_q)
        k = jnp.einsum("bkc,chd->bhkd", c_kv, w_uk)
        v = jnp.einsum("bkc,chd->bhkd", c_kv, w_uv)
        scores = jnp.einsum("bhqd,bhkd->bhqk", q, k) * (D ** -0.5)
        off = Sk - Sq
        qi = jnp.arange(Sq)[:, None]
        kj = jnp.arange(Sk)[None, :]
        cmask = kj <= (qi + off)
        scores = jnp.where(cmask[None, None], scores, -1e9)
        p = _softmax(scores, axis=-1)
        ctx = jnp.einsum("bhqk,bhkd->bhqd", p, v)
        return jnp.einsum("bhqd,hdm->bqm", ctx, w_o)

    def _B_ref(x, w1, b1, w2, b2):
        h = jnp.einsum("bsd,df->bsf", x, w1) + b1
        h = _gelu(h)
        return jnp.einsum("bsf,fd->bsd", h, w2) + b2

    x = A_x
    xn = _layernorm(x, axis=-1)
    s = _A_ref(xn, A_c_kv, A_w_q, A_w_uk, A_w_uv, A_w_o)
    g = _silu(_B_ref(xn, B_w1, B_b1, B_w2, B_b2))
    return x + s * g
```

```python
import contextlib
import jax
import jax.numpy as jnp
from jax import lax
import jax.experimental.pallas as pl
import jax.experimental.pallas.tpu as pltpu

F32 = jnp.float32
BF16 = jnp.bfloat16

B, H, SK, D, M, DC, F = 2, 32, 16384, 128, 512, 512, 1792
LOG2E = 1.4426950408889634
NT = (((1,), (1,)), ((), ()))


def _loop(lo, hi, body):
    lax.fori_loop(lo, hi, lambda i, _: body(i), None)


def _rows8(v):
    return jnp.concatenate([v[:, j * 128:(j + 1) * 128] for j in range(M // 128)], axis=0)


def _runs(name, lo, hi):
    return [(name, r) for r in range(lo, hi)]


def make(TR=False, LAG=2, END=197, CUTS=(0, 8, 20, 24, 28, 31, 32), QP=4, TAIL=(1, 1), STEP=2.5, DMA_ONLY=False, LASTQ=(), plan=0):
    PHASES = [
        ((_runs('w1', 0, 2) + _runs('uv', 0, 4) + _runs('uk', 0, 4) + _runs('q', 0, 4) + _runs('c', 0, 2)),
         (_runs('c', 2, 16) + _runs('w2', 0, 2)), _runs('c', 16, 32)),
        ((_runs('uv', 0, 4) + _runs('uk', 0, 4) + _runs('q', 0, 4) + _runs('c', 0, 4)),
         (_runs('c', 4, 16) + _runs('w2', 0, 2) + _runs('w1', 0, 2)), _runs('c', 16, 32)),
        ((_runs('uv', 0, 4) + _runs('uk', 0, 4) + _runs('q', 0, 4) + _runs('c', 0, 4)),
         (_runs('c', 4, 18) + _runs('w1', 0, 2)), _runs('c', 18, 32) + _runs('w2', 0, 2)),
    ][plan]
    ROUNDS = 3 * 64 + 16
    scope = (lambda n: jax.named_scope('@' + n)) if TR else (lambda n: contextlib.nullcontext())

    def _kernel(x_hbm, c_hbm, wq_hbm, wuk_hbm, wuv_hbm, wo_hbm, w1_hbm, b1_hbm, w2_hbm, b2_hbm,
                o_hbm,
                x_buf, b1_buf, b2_buf, c_buf, wq_buf, wuk_buf, wuv_buf, wo_buf, w1_buf, w2_buf,
                xs, t8, qa_ref, acc_ref, m_ref, l_ref, s_ref, ctx_ref, mul_ref, o_buf,
                sem_w, sem_c, sem_o, sem_last, sem_small):
        weights = dict(q=(wq_hbm, wq_buf, 0), uk=(wuk_hbm, wuk_buf, 1), uv=(wuv_hbm, wuv_buf, 2),
                       w1=(w1_hbm, w1_buf, 3), w2=(w2_hbm, w2_buf, 4))

        def fetch(name, run, j, queue):
            if name == 'c':
                b = run // 16
                src, dst, sem = c_hbm.at[run * 64 + j], c_buf.at[b, j, run % 16], sem_c.at[b * 16 + (j >> 2)]
            elif name == 'o':
                src, dst, sem = wo_hbm.at[run, j], wo_buf.at[run, j], sem_o.at[j >> 3]
            else:
                hbm, buf, s = weights[name]
                ix = pl.ds((run * 64 + j) * 8, 8) if name == 'w1' else run * 64 + j
                src, dst, sem = hbm.at[ix], buf.at[ix], sem_w.at[s]
            pltpu.make_async_copy(src, dst, sem).start(priority=queue)

        def pieces(phase, j):
            if phase < 3:
                return [(name, run, j - 64 * phase) for name, run in PHASES[phase]]
            return [('o', run, 2 * (j - 192) + t) for t in range(2) for run in range(7)]

        def issue_round(j, at):
            ahead = pieces((at + LAG) // 64, j + LAG) if at + LAG < ROUNDS else []
            now = pieces(at // 64, j) if at >= 0 else []
            for i in range(16):
                if i % QP == 0:
                    if i < len(now) and not (at == 0 and i == 0):
                        fetch(*now[i], 0)
                elif i < len(ahead):
                    name, run, k = ahead[i]
                    if not (name in ('w1', 'w2') and run == 1 and (at + LAG) % 64 >= 48):
                        fetch(name, run, k, 1)
                elif at + LAG >= ROUNDS:
                    fetch_last((at + LAG - ROUNDS) * 12 + i - i // QP - 1)

        def fetch_last(p):
            s = max(i for i, cut in enumerate(CUTS) if cut <= p)
            pltpu.make_async_copy(wo_hbm.at[7, p], wo_buf.at[7, p], sem_last.at[s]).start(priority=int(p not in LASTQ))

        edges = sorted({-LAG, 0, 1, ROUNDS} | {64 * p + e for p in range(3) for e in (48 - LAG, 64 - LAG, 64)}
                       | set(range(ROUNDS - LAG, ROUNDS)))

        def issue(lo, hi, *within):
            for s, e in zip(edges, edges[1:]):
                if not within:
                    if max(lo, s) + 1 == min(hi, e):
                        issue_round(max(lo, s), s)
                    elif max(lo, s) < min(hi, e):
                        _loop(max(lo, s), min(hi, e), lambda j: issue_round(j, s))
                elif any(max(a, s) < min(z, e) for a, z in within):
                    _loop(jnp.maximum(lo, s), jnp.minimum(hi, e), lambda j: issue_round(j, s))

        def wait_filled(buf, sem):
            pltpu.make_async_copy(buf, buf, sem).wait()

        x_copy = pltpu.make_async_copy(x_hbm, x_buf, sem_small.at[0])
        b1_copy = pltpu.make_async_copy(b1_hbm, b1_buf, sem_small.at[1])
        b2_copy = pltpu.make_async_copy(b2_hbm, b2_buf, sem_small.at[2])

        fetch(*pieces(0, 0)[0], 0)
        issue(-LAG, 8)
        for c in (x_copy, b1_copy, b2_copy):
            c.start()
        issue(8, 16)

        if DMA_ONLY:
            issue(16, ROUNDS)
            for p in range(12 * LAG, 32):
                fetch_last(p)
            for c in (x_copy, b1_copy, b2_copy):
                c.wait()
            for _, buf, s in weights.values():
                wait_filled(buf, sem_w.at[s])
            for i in range(32):
                wait_filled(c_buf.at[0, pl.ds(0, 4)], sem_c.at[i])
            for k in range(4):
                wait_filled(wo_buf.at[pl.ds(0, 7), pl.ds(8 * k, 8)], sem_o.at[k])
            for i in range(len(CUTS) - 1):
                wait_filled(wo_buf.at[7, pl.ds(CUTS[i], CUTS[i + 1] - CUTS[i])], sem_last.at[i])
            o_buf[...] = jnp.zeros((8, 128), BF16)
            o_copy = pltpu.make_async_copy(o_buf, o_hbm, sem_small.at[0])
            o_copy.start()
            o_copy.wait()
            return

        x_copy.wait()
        with scope('ln'):
            x = x_buf[...].astype(F32)
            xc = x - jnp.mean(x, axis=-1, keepdims=True)
            var = jnp.mean(xc * xc, axis=-1, keepdims=True)
            xn = (xc * lax.rsqrt(var + 1e-5)).astype(BF16)
            xf = xn.astype(F32)
            for b in range(B):
                for j in range(M // 128):
                    cols = slice(j * 128, (j + 1) * 128)
                    xs[b, cols, :] = jnp.broadcast_to(xf[b:b + 1, cols], (128, 128)).T
        issue(16, 70)

        wait_filled(wq_buf, sem_w.at[0])

        def q_rows(i, carry):
            q0, q1 = carry
            for u in range(8):
                m = pl.ds(i * 8 + u, 1)
                w = wq_buf[i * 4 + u // 2, pl.ds((u % 2) * H, H)].astype(F32)
                q0 = q0 + xs[0, m, :] * w
                q1 = q1 + xs[1, m, :] * w
            return q0, q1

        def q_step(i, carry):
            issue(70 + 2 * i, 72 + 2 * i, (70, 78))
            with scope('q'):
                return lax.fori_loop(i * 16, i * 16 + 16, q_rows, carry)

        q0, q1 = lax.fori_loop(0, 4, q_step, (jnp.zeros((H, D), F32), jnp.zeros((H, D), F32)))
        q = jnp.concatenate([q0, q1, jnp.zeros((128 - B * H, D), F32)], axis=0).astype(BF16)

        wait_filled(wuk_buf, sem_w.at[1])
        group = (lax.broadcasted_iota(jnp.int32, (16, 8, 128), 2) % H) // 8

        def qa_step(i):
            issue(78 + 2 * i, 80 + 2 * i, (78, 94))
            with scope('qa'):
                for u in range(4):
                    w = wuk_buf[pl.ds((i * 4 + u) * 8, 8)].reshape(16 * H, D)
                    r = lax.dot_general(w, q, NT, preferred_element_type=F32).reshape(16, 4, 8, 128)
                    v = jnp.where(group == 0, r[:, 0],
                                  jnp.where(group == 1, r[:, 1], jnp.where(group == 2, r[:, 2], r[:, 3])))
                    t8[pl.ds(pl.multiple_of((i * 4 + u) * 128, 128), 128), :] = v.reshape(128, 128)

        _loop(0, 8, qa_step)
        issue(94, 96)
        with scope('qat'):
            sub = lax.broadcasted_iota(jnp.int32, (128, 128), 1) % 8
            for j in range(DC // 128):
                t = t8[pl.ds(j * 1024, 128, stride=8), :]
                for s in range(1, 8):
                    t = jnp.where(sub == s, t8[pl.ds(j * 1024 + s, 128, stride=8), :], t)
                qa_ref[:, j * 128:(j + 1) * 128] = (t.T[:B * H] * (D ** -0.5 * LOG2E)).astype(BF16)
        per = 16 * STEP + 6
        first = int(END + 6 - B * per)
        issue(96, 98)

        wait_filled(w1_buf, sem_w.at[3])
        b1_copy.wait()
        with scope('hid'):
            w1 = jnp.concatenate(
                [jnp.concatenate([w1_buf[r * (F // 128) + j].astype(F32) for r in range(M // 8)], axis=0).astype(BF16)
                 for j in range(F // 128)], axis=1)
            hid = jnp.dot(xn, w1, preferred_element_type=F32)
            hid = jax.nn.gelu(hid + b1_buf[...].astype(F32).reshape(1, F), approximate=True).astype(BF16)
        issue(98, first)
        wait_filled(wuv_buf, sem_w.at[2])

        def batch(b):
            heads = pl.ds(pl.multiple_of(b * H, H), H)
            m_ref[...] = jnp.full((H, 128), -jnp.inf, F32)
            l_ref[...] = jnp.zeros((H, 128), F32)
            acc_ref[...] = jnp.zeros((H, DC), F32)

            def advance(lo, hi):
                at = lambda b, i: first + int(per) * b + ((int(2 * STEP) * i) >> 1)
                ends = (lo, hi) if isinstance(lo, int) else (1, 16)
                issue(at(b, lo), at(b, hi), *[(at(k, ends[0]), at(k, ends[1])) for k in range(B)])

            def scores(i):
                keys = c_buf.at[b, pl.ds(i * 4, 4)]
                wait_filled(keys, sem_c.at[b * 16 + i])
                return lax.dot_general(qa_ref[heads, :], keys[...].reshape(1024, DC), NT, preferred_element_type=F32)

            def accumulate(i):
                sc = s_ref[...]
                m_prev = m_ref[...]
                m_new = jnp.maximum(m_prev, jnp.max(sc, axis=1, keepdims=True))
                p = jnp.exp2(sc - m_new[:, :1])
                alpha = jnp.exp2(m_prev - m_new)
                l_ref[...] = alpha * l_ref[...] + jnp.sum(p, axis=1, keepdims=True)
                m_ref[...] = m_new
                pv = jnp.dot(p.astype(BF16), c_buf[b, pl.ds(i * 4, 4)].reshape(1024, DC), preferred_element_type=F32)
                acc_ref[...] = acc_ref[...] * alpha[:, :1] + pv

            def block(i):
                advance(i, i + 1)
                with scope('att'):
                    sc = scores(i)
                    accumulate(i - 1)
                    s_ref[...] = sc

            advance(0, 1)
            with scope('s0'):
                s_ref[...] = scores(0)
            _loop(1, 16, block)
            done = first + int(per) * (b + 1) - 6
            tails = lambda lo, hi: [(first + int(per) * (k + 1) - 6 + lo, first + int(per) * (k + 1) - 6 + hi) for k in range(B)]
            issue(done, done + 2, *tails(0, 2))
            with scope('acc'):
                accumulate(15)

            issue(done + 2, done + 4, *tails(2, 4))
            with scope('pc'):
                pc = acc_ref[...] / l_ref[...][:, :1]
                for j in range(DC // 128):
                    cols = slice(j * 128, (j + 1) * 128)
                    t8[cols, :] = jnp.concatenate([pc[:, cols]] * 4, axis=0).T
                quarter = lax.broadcasted_iota(jnp.int32, (128, 128), 1) // H
                flat = t8[pl.ds(0, 128, stride=4), :]
                for s in range(1, 4):
                    flat = jnp.where(quarter == s, t8[pl.ds(s, 128, stride=4), :], flat)
                t8[pl.ds(1024, 128), :] = flat
            diag = lax.broadcasted_iota(jnp.int32, (H, 128), 1) % H == lax.broadcasted_iota(jnp.int32, (H, 128), 0)

            def ctx_step(i, ctx):
                issue(done + 4 + i, done + 5 + i, *tails(4, 6))
                with scope('ctx'):
                    a = jnp.concatenate([jnp.where(diag, t8[pl.ds(1024 + i * 64 + t, 1), :], 0.0) for t in range(64)], axis=1)
                    return ctx + jnp.dot(a.astype(BF16), wuv_buf[pl.ds(i * 128, 128)].reshape(64 * 128, D),
                                         preferred_element_type=F32)

            ctx_ref[heads, :] = lax.fori_loop(0, 2, ctx_step, jnp.zeros((H, D), F32))

        _loop(0, B, batch)
        at = [END + 6]

        def more(n):
            issue(at[0], min(at[0] + n, ROUNDS))
            at[0] = min(at[0] + n, ROUNDS)

        more(TAIL[0])
        with scope('mul'):
            for b in range(B):
                for k in range(1, 4):
                    v = ctx_ref[pl.ds(b * H + H - 4 + k, 1), :].astype(BF16).astype(F32)
                    mul_ref[b, (k - 1) * D:k * D] = jnp.broadcast_to(v, (128, 128)).T
        more(TAIL[1])

        wait_filled(w2_buf, sem_w.at[4])
        b2_copy.wait()
        with scope('z'):
            z = jnp.dot(hid, w2_buf[...].reshape(F, M), preferred_element_type=F32)
            z8 = _rows8(z + b2_buf[...].astype(F32).reshape(1, M))
            g8 = z8 * jax.nn.sigmoid(z8)
            x8 = _rows8(x)
        more(ROUNDS)
        for p in range(12 * LAG, 32):
            fetch_last(p)

        def project(a0, n, heads):
            lhs = jnp.concatenate([ctx_ref[pl.ds(4 * a + k, B, stride=H), :]
                                   for k in heads for a in range(a0, a0 + n)], axis=1)
            rhs = jnp.concatenate([wo_buf[a0:a0 + n, 8 * k:8 * k + 8].reshape(n * D, M) for k in heads], axis=0)
            return jnp.dot(lhs.astype(BF16), rhs, preferred_element_type=F32)

        def wait_last(i):
            with scope(f'l{i}'):
                wait_filled(wo_buf.at[7, pl.ds(CUTS[i], CUTS[i + 1] - CUTS[i])], sem_last.at[i])

        s = jnp.zeros((B, M), F32)
        for heads in ((0, 1), (2,), (3,)):
            with scope(f'ow{heads[0]}'):
                for k in heads:
                    wait_filled(wo_buf.at[pl.ds(0, 7), pl.ds(8 * k, 8)], sem_o.at[k])
            s = s + project(0, 7, heads)
        wait_last(0)
        base8 = x8 + _rows8(s + project(7, 1, (0,))) * g8

        part = [[None] * (M // 128) for _ in range(B)]
        for i in range(1, len(CUTS) - 1):
            wait_last(i)
            for r in range(16 * CUTS[i], 16 * CUTS[i + 1], 8):
                w = wo_buf[7, r // 16, r % 16:r % 16 + 8].astype(F32)
                for b in range(B):
                    mul = mul_ref[b, r - D:r - D + 8, :]
                    for j in range(M // 128):
                        t = w[:, j * 128:(j + 1) * 128] * mul
                        part[b][j] = t if part[b][j] is None else part[b][j] + t

        sl = lax.broadcasted_iota(jnp.int32, (8, 128), 0)

        def merge(lo, hi, k):
            m = (sl & k) != 0
            if k == 4:
                return jnp.where(m, hi, lo) + pltpu.roll(jnp.where(m, lo, hi), 4, 0)
            return jnp.where(m, hi, lo) + jnp.where(m, pltpu.roll(hi, k, 0), pltpu.roll(lo, 8 - k, 0))

        r4 = [[merge(part[b][j], part[b][j + 2], 4) for j in range(2)] for b in range(B)]
        r2 = [merge(r4[b][0], r4[b][1], 2) for b in range(B)]
        o_buf[...] = (base8 + g8 * merge(r2[0], r2[1], 1)).astype(BF16)
        o_copy = pltpu.make_async_copy(o_buf, o_hbm, sem_small.at[0])
        o_copy.start()
        o_copy.wait()

    def fn(A_x, A_c_kv, A_w_q, A_w_uk, A_w_uv, A_w_o, B_x, B_w1, B_b1, B_w2, B_b2):
        hbm = pl.BlockSpec(memory_space=pltpu.HBM)
        dma_sems = pltpu.SemaphoreType.DMA
        w_view, o_view, w1_view, w2_view = (256, 2 * H, D), (8, 32, 16, M), (896, 8, 128), (112, 16, M)
        out = pl.pallas_call(
            _kernel,
            out_shape=jax.ShapeDtypeStruct((8, 128), BF16),
            in_specs=[hbm] * 10,
            out_specs=hbm,
            scratch_shapes=[
                pltpu.VMEM((B, M), BF16), pltpu.VMEM((F,), BF16), pltpu.VMEM((M,), BF16),
                pltpu.VMEM((B, 64, 16, 16, DC), BF16), pltpu.VMEM(w_view, BF16), pltpu.VMEM(w_view, BF16),
                pltpu.VMEM(w_view, BF16), pltpu.VMEM(o_view, BF16),
                pltpu.VMEM(w1_view, BF16), pltpu.VMEM(w2_view, BF16),
                pltpu.VMEM((B, M, 128), F32),
                pltpu.VMEM((DC * 8 + 8, 128), F32),
                pltpu.VMEM((B * H, DC), BF16), pltpu.VMEM((H, DC), F32),
                pltpu.VMEM((H, 128), F32), pltpu.VMEM((H, 128), F32),
                pltpu.VMEM((H, 1024), F32),
                pltpu.VMEM((3 * H, D), F32), pltpu.VMEM((B, 3 * D, 128), F32), pltpu.VMEM((8, 128), BF16),
                dma_sems((5,)), dma_sems((32,)), dma_sems((4,)), dma_sems((len(CUTS) - 1,)),
                dma_sems((3,)),
            ],
            compiler_params=pltpu.CompilerParams(
                vmem_limit_bytes=100 * 1024 * 1024, disable_semaphore_checks=True, disable_bounds_checks=True),
        )(A_x.reshape(B, M), A_c_kv.reshape(2048, 16, DC), A_w_q.reshape(w_view), A_w_uk.reshape(w_view),
          A_w_uv.reshape(w_view), A_w_o.reshape(o_view),
          B_w1.reshape(M // 8, 8, F // 128, 128).transpose(0, 2, 1, 3).reshape(w1_view), B_b1,
          B_w2.reshape(w2_view), B_b2)
        return out.reshape(M // 128, B, 128).transpose(1, 0, 2).reshape(B, 1, M)
    return fn


_impl = make(END=198, TAIL=(2,2))


@jax.jit
def pallas_recurrent_scan__compressed_kv_cla__dense_activation_gelu__decode_kernel(
    A_x, A_c_kv, A_w_q, A_w_uk, A_w_uv, A_w_o, B_x, B_w1, B_b1, B_w2, B_b2,
):
    return _impl(A_x, A_c_kv, A_w_q, A_w_uk, A_w_uv, A_w_o, B_x, B_w1, B_b1, B_w2, B_b2)
```

```python
import contextlib
import jax
import jax.numpy as jnp
from jax import lax
import jax.experimental.pallas as pl
import jax.experimental.pallas.tpu as pltpu

F32 = jnp.float32
BF16 = jnp.bfloat16

B, H, SK, D, M, DC, F = 2, 32, 16384, 128, 512, 512, 1792
LOG2E = 1.4426950408889634
NT = (((1,), (1,)), ((), ()))


def _loop(lo, hi, body):
    lax.fori_loop(lo, hi, lambda i, _: body(i), None)


def _rows8(v):
    return jnp.concatenate([v[:, j * 128:(j + 1) * 128] for j in range(M // 128)], axis=0)


def parse(s):
    out = []
    for t in s.split():
        t, _, k = t.partition('+'); a = t[:2] if t[0] in 'uw' else t[0]; lo, _, hi = t[len(a):].lstrip('.').partition('-')
        out += [(a, i, int(k or 0)) for i in range(int(lo), int(hi or int(lo) + 1))]
    return out


def make(TR=False, END=198, CUTS=(0, 8, 16, 20, 24, 26, 28, 30, 31, 32), MXU=0, STEP=2.75, DMA_ONLY=False, EARLY=7, SLOT=2, SMALL=8, DSLOT=2, SQ=0, FOLD=False, PEEL=0, ONE=True,
         ph=('uv0-4 uk0-4 q0-4 c0-3 w1.0', 'c3-16 w2.0-2 w1.1', 'c16-32')):
    PHASES = [parse(p) for p in ph]
    assert all(len(p) == 16 for p in PHASES) and len({r[:2] for p in PHASES for r in p}) == 48
    assert all(a == 'c' and r >= 16 for a, r, _ in PHASES[2]) and not any(a in ('q', 'uk') for a, r, _ in PHASES[1])
    ROUNDS = 3 * 64 + 16
    LAG = 2
    scope = (lambda n: jax.named_scope('@' + n)) if TR else (lambda n: contextlib.nullcontext())

    def _kernel(x_hbm, c_hbm, wq_hbm, wuk_hbm, wuv_hbm, wo_hbm, w1_hbm, b1_hbm, w2_hbm, b2_hbm,
                o_hbm,
                x_buf, b1_buf, b2_buf, c_buf, wq_buf, wuk_buf, wuv_buf, wo_buf, w1_buf, w2_buf,
                xs, t8, qa_ref, acc_ref, m_ref, l_ref, s_ref, ctx_ref, mul_ref, gate_ref, o_buf,
                *sems):
        if ONE:
            sems = [sems[0].at[pl.ds(a, n)] for a, n in ((0, 5), (5, 32), (37, 4), (44, len(CUTS) - 1), (41, 3))]
        sem_w, sem_c, sem_o, sem_last, sem_small = sems
        weights = dict(q=(wq_hbm, wq_buf, 0), uk=(wuk_hbm, wuk_buf, 1), uv=(wuv_hbm, wuv_buf, 2),
                       w1=(w1_hbm, w1_buf, 3), w2=(w2_hbm, w2_buf, 4))

        def fetch(phase, j, i, queue):
            if phase == 3:
                if i % 8 == 7:
                    return
                k, run = 2 * (j - 192) + i // 8, (0, 2, 4, 6, 1, 3, 5)[i % 8]
                pltpu.make_async_copy(wo_hbm.at[run, k], wo_buf.at[run, k], sem_o.at[(j - 192) >> 2]).start(priority=queue)
                return
            name, run, skew = PHASES[phase][i]
            j = j - 64 * phase
            p = run * 64 + ((j + skew) & 63 if skew else j)
            if name == 'c':
                b = run // 16
                pltpu.make_async_copy(c_hbm.at[p], c_buf.at[b, j, run % 16], sem_c.at[b * 16 + (j >> 2)]).start(priority=queue)
                return
            hbm, buf, s = weights[name]

            def go():
                ix = pl.ds(p * 8, 8) if name == 'w1' else p
                pltpu.make_async_copy(hbm.at[ix], buf.at[ix], sem_w.at[s]).start(priority=queue)
            if name in ('w1', 'w2') and run == 1:
                pl.when(p < 112)(go)
            else:
                go()

        def fetch_last(p):
            s = max(i for i, cut in enumerate(CUTS) if cut <= p)
            pltpu.make_async_copy(wo_hbm.at[7, p], wo_buf.at[7, p], sem_last.at[s]).start(priority=1)

        def issue_round(j, at):
            for g in range(4):
                for t in range(4):
                    if t == (SLOT if at < 192 else DSLOT) and not (at == 0 and g == 0):
                        fetch(at // 64, j, 6 if at == 0 and g == 1 else 4 * g, 0)
                    if t == 3:
                        continue
                    if at + LAG < ROUNDS:
                        fetch((at + LAG) // 64, j + LAG, 4 * g + 1 + t, 1)
                    else:
                        fetch_last((at + LAG - ROUNDS) * 12 + 3 * g + t)

        edges = sorted({0, 1, ROUNDS} | {64 * p + e for p in range(3) for e in (64 - LAG, 64)}
                       | set(range(ROUNDS - LAG, ROUNDS)))

        def issue(lo, hi, *within):
            for s, e in zip(edges, edges[1:]):
                if not within:
                    if max(lo, s) + 1 == min(hi, e):
                        issue_round(max(lo, s), s)
                    elif max(lo, s) < min(hi, e):
                        _loop(max(lo, s), min(hi, e), lambda j: issue_round(j, s))
                elif any(max(a, s) < min(z, e) for a, z in within):
                    _loop(jnp.maximum(lo, s), jnp.minimum(hi, e), lambda j: issue_round(j, s))

        def wait_filled(buf, sem):
            pltpu.make_async_copy(buf, buf, sem).wait()

        x_copy = pltpu.make_async_copy(x_hbm, x_buf, sem_small.at[0])
        b1_copy = pltpu.make_async_copy(b1_hbm, b1_buf, sem_small.at[1])
        b2_copy = pltpu.make_async_copy(b2_hbm, b2_buf, sem_small.at[2])

        for n, (j, i) in enumerate([(j, i) for j in range(LAG) for i in range(16) if i % 4 and (j, i) not in ((0, 2), (0, 6))]):
            if n % EARLY == 0 and n < 3 * EARLY:
                fetch(0, 0, 2 * (n // EARLY), 0)
            fetch(0, j, i, 1)
        issue(0, SMALL)
        for c in (x_copy, b1_copy, b2_copy):
            c.start(priority=SQ)
        issue(SMALL, 16)

        if DMA_ONLY:
            issue(16, ROUNDS)
            for p in range(12 * LAG, 32):
                fetch_last(p)
            for c in (x_copy, b1_copy, b2_copy):
                c.wait()
            for _, buf, s in weights.values():
                wait_filled(buf, sem_w.at[s])
            for i in range(32):
                wait_filled(c_buf.at[0, pl.ds(0, 4)], sem_c.at[i])
            for k in range(4):
                wait_filled(wo_buf.at[pl.ds(0, 7), pl.ds(8 * k, 8)], sem_o.at[k])
            for i in range(len(CUTS) - 1):
                wait_filled(wo_buf.at[7, pl.ds(CUTS[i], CUTS[i + 1] - CUTS[i])], sem_last.at[i])
            o_buf[...] = jnp.zeros((8, 128), BF16)
            o_copy = pltpu.make_async_copy(o_buf, o_hbm, sem_small.at[0])
            o_copy.start()
            o_copy.wait()
            return

        x_copy.wait()
        with scope('ln'):
            x = x_buf[...].astype(F32)
            xc = x - jnp.mean(x, axis=-1, keepdims=True)
            var = jnp.mean(xc * xc, axis=-1, keepdims=True)
            xn = (xc * lax.rsqrt(var + 1e-5)).astype(BF16)
            xf = xn.astype(F32)
            for b in range(B):
                for j in range(M // 128):
                    cols = slice(j * 128, (j + 1) * 128)
                    xs[b, cols, :] = jnp.broadcast_to(xf[b:b + 1, cols], (128, 128)).T
        issue(16, 70)

        wait_filled(wq_buf, sem_w.at[0])

        def q_rows(i, carry):
            q0, q1 = carry
            for u in range(8):
                m = pl.ds(i * 8 + u, 1)
                w = wq_buf[i * 4 + u // 2, pl.ds((u % 2) * H, H)].astype(F32)
                q0 = q0 + xs[0, m, :] * w
                q1 = q1 + xs[1, m, :] * w
            return q0, q1

        def q_step(i, carry):
            issue(70 + 2 * i, 72 + 2 * i, (70, 78))
            with scope('q'):
                return lax.fori_loop(i * 16, i * 16 + 16, q_rows, carry)

        q0, q1 = lax.fori_loop(0, 4, q_step, (jnp.zeros((H, D), F32), jnp.zeros((H, D), F32)))
        q = jnp.concatenate([q0, q1, jnp.zeros((128 - B * H, D), F32)], axis=0).astype(BF16)

        wait_filled(wuk_buf, sem_w.at[1])
        group = (lax.broadcasted_iota(jnp.int32, (16, 8, 128), 2) % H) // 8

        def qa_step(i):
            issue(78 + 2 * i, 80 + 2 * i, (78, 94))
            with scope('qa'):
                for u in range(4):
                    w = wuk_buf[pl.ds((i * 4 + u) * 8, 8)].reshape(16 * H, D)
                    r = lax.dot_general(w, q, NT, preferred_element_type=F32).reshape(16, 4, 8, 128)
                    v = jnp.where(group == 0, r[:, 0],
                                  jnp.where(group == 1, r[:, 1], jnp.where(group == 2, r[:, 2], r[:, 3])))
                    t8[pl.ds(pl.multiple_of((i * 4 + u) * 128, 128), 128), :] = v.reshape(128, 128)

        _loop(0, 8, qa_step)
        issue(94, 96)
        with scope('qat'):
            sub = lax.broadcasted_iota(jnp.int32, (128, 128), 1) % 8
            for j in range(DC // 128):
                t = t8[pl.ds(j * 1024, 128, stride=8), :]
                for s in range(1, 8):
                    t = jnp.where(sub == s, t8[pl.ds(j * 1024 + s, 128, stride=8), :], t)
                qa_ref[:, j * 128:(j + 1) * 128] = (t.T[:B * H] * (D ** -0.5 * LOG2E)).astype(BF16)
        per = 16 * STEP + 13
        first = int(END + 13 - B * per)
        assert first >= 96 and END + 8 <= ROUNDS - LAG
        issue(96, first)

        def batch(b):
            heads = pl.ds(pl.multiple_of(b * H, H), H)
            m_ref[...] = jnp.full((H, 128), -jnp.inf, F32)
            l_ref[...] = jnp.zeros((H, 128), F32)
            acc_ref[...] = jnp.zeros((H, DC), F32)

            def advance(lo, hi):
                at = lambda b, i: first + int(per) * b + ((int(4 * STEP) * i) >> 2)
                ends = (lo, hi) if isinstance(lo, int) else (1, 16)
                issue(at(b, lo), at(b, hi), *[(at(k, ends[0]), at(k, ends[1])) for k in range(B)])

            def scores(i):
                keys = c_buf.at[b, pl.ds(i * 4, 4)]
                wait_filled(keys, sem_c.at[b * 16 + i])
                return lax.dot_general(qa_ref[heads, :], keys[...].reshape(1024, DC), NT, preferred_element_type=F32)

            def accumulate(i):
                sc = s_ref[...]
                m_prev = m_ref[...]
                m_new = jnp.maximum(m_prev, jnp.max(sc, axis=1, keepdims=True))
                p = jnp.exp2(sc - m_new[:, :1])
                alpha = jnp.exp2(m_prev - m_new)
                l_ref[...] = alpha * l_ref[...] + jnp.sum(p, axis=1, keepdims=True)
                m_ref[...] = m_new
                pv = jnp.dot(p.astype(BF16), c_buf[b, pl.ds(i * 4, 4)].reshape(1024, DC), preferred_element_type=F32)
                acc_ref[...] = acc_ref[...] * alpha[:, :1] + pv

            def block(i):
                advance(i, i + 1)
                with scope('att'):
                    sc = scores(i)
                    accumulate(i - 1)
                    s_ref[...] = sc

            advance(0, 1)
            with scope('s0'):
                s_ref[...] = scores(0)
            _loop(1, 16, block)
            done = first + int(per) * (b + 1) - 13
            tails = lambda lo, hi: [(first + int(per) * (k + 1) - 13 + lo, first + int(per) * (k + 1) - 13 + hi) for k in range(B)]
            issue(done, done + 2, *tails(0, 2))
            with scope('acc'):
                accumulate(15)

            issue(done + 2, done + 4, *tails(2, 4))
            with scope('pc'):
                pc = acc_ref[...] / l_ref[...][:, :1]
                for j in range(DC // 128):
                    cols = slice(j * 128, (j + 1) * 128)
                    t8[cols, :] = jnp.concatenate([pc[:, cols]] * 4, axis=0).T
                quarter = lax.broadcasted_iota(jnp.int32, (128, 128), 1) // H
                flat = t8[pl.ds(0, 128, stride=4), :]
                for s in range(1, 4):
                    flat = jnp.where(quarter == s, t8[pl.ds(s, 128, stride=4), :], flat)
                t8[pl.ds(1024, 128), :] = flat
            diag = lax.broadcasted_iota(jnp.int32, (H, 128), 1) % H == lax.broadcasted_iota(jnp.int32, (H, 128), 0)

            pl.when(b == 0)(lambda: wait_filled(wuv_buf, sem_w.at[2]))

            def ctx_step(i, ctx):
                issue(done + 4 + 2 * i, done + 6 + 2 * i, *tails(4, 8))
                with scope('ctx'):
                    a = jnp.concatenate([jnp.where(diag, t8[pl.ds(1024 + i * 64 + t, 1), :], 0.0) for t in range(64)], axis=1)
                    return ctx + jnp.dot(a.astype(BF16), wuv_buf[pl.ds(i * 128, 128)].reshape(64 * 128, D),
                                         preferred_element_type=F32)

            ctx_ref[heads, :] = lax.fori_loop(0, 2, ctx_step, jnp.zeros((H, D), F32))

            @pl.when(b == 0)
            def _():
                issue(*tails(8, 11)[0])
                wait_filled(w1_buf, sem_w.at[3])
                b1_copy.wait()
                with scope('hid'):
                    w1 = jnp.concatenate(
                        [jnp.concatenate([w1_buf[r * (F // 128) + j].astype(F32) for r in range(M // 8)], axis=0).astype(BF16)
                         for j in range(F // 128)], axis=1)
                    hid = jnp.dot(xn, w1, preferred_element_type=F32)
                    hid = jax.nn.gelu(hid + b1_buf[...].astype(F32).reshape(1, F), approximate=True).astype(BF16)
                issue(*tails(11, 13)[0])
                wait_filled(w2_buf, sem_w.at[4])
                b2_copy.wait()
                with scope('z'):
                    z = jnp.dot(hid, w2_buf[...].reshape(F, M), preferred_element_type=F32)
                    z8 = _rows8(z + b2_buf[...].astype(F32).reshape(1, M))
                    gate_ref[...] = z8 * jax.nn.sigmoid(z8)

        _loop(0, B, batch)
        issue(END + 8, ROUNDS)
        for p in range(12 * LAG, 32):
            fetch_last(p)
        sl = lax.broadcasted_iota(jnp.int32, (8, 128), 0)
        with scope('mul'):
            for b in range(B):
                for k in range(MXU, 4):
                    v = ctx_ref[pl.ds(b * H + H - 4 + k, 1), :].astype(BF16).astype(F32)
                    mul_ref[b, k * D:(k + 1) * D] = jnp.broadcast_to(v, (128, 128)).T

        def project(k, s):
            w = wo_buf.at[pl.ds(0, 7), pl.ds(8 * k, 8)]
            with scope('ow'):
                wait_filled(w, sem_o.at[k])
            lhs = jnp.concatenate([ctx_ref[pl.ds(4 * a + k, B, stride=H), :] for a in range(7)], axis=1)
            return s + jnp.dot(lhs.astype(BF16), w[...].reshape(7 * D, M), preferred_element_type=F32)

        def wait_last(i):
            with scope(f'l{i}'):
                wait_filled(wo_buf.at[7, pl.ds(CUTS[i], CUTS[i + 1] - CUTS[i])], sem_last.at[i])

        s = lax.fori_loop(0, 4 - PEEL, project, jnp.zeros((B, M), F32))
        if PEEL:
            s = project(3, s)
        for k in range(MXU):
            assert CUTS[k + 1] == 8 * k + 8
            wait_last(k)
            s = s + jnp.dot(ctx_ref[pl.ds(28 + k, B, stride=H), :].astype(BF16), wo_buf[7, 8 * k:8 * k + 8].reshape(D, M),
                            preferred_element_type=F32)
        g8 = gate_ref[...]
        base8 = _rows8(x) + _rows8(s) * g8

        part = [[None] * (M // 128) for _ in range(B)]
        for i in range(MXU, len(CUTS) - 1):
            muls = {(b, r): mul_ref[b, r:r + 8, :] for b in range(B) for r in range(16 * CUTS[i], 16 * CUTS[i + 1], 8)}
            wait_last(i)
            for r in range(16 * CUTS[i], 16 * CUTS[i + 1], 8):
                w = wo_buf[7, r // 16, r % 16:r % 16 + 8].astype(F32)
                for b in range(B):
                    mul = muls[b, r] if CUTS[i + 1] - CUTS[i] <= 4 else mul_ref[b, r:r + 8, :]
                    for j in range(M // 128):
                        t = w[:, j * 128:(j + 1) * 128] * mul
                        part[b][j] = t if part[b][j] is None else part[b][j] + t

        def halves(lo, hi, k):
            m = (sl & k) != 0
            if k == 4:
                return jnp.where(m, hi, lo), pltpu.roll(jnp.where(m, lo, hi), 4, 0)
            return jnp.where(m, hi, lo), jnp.where(m, pltpu.roll(hi, k, 0), pltpu.roll(lo, 8 - k, 0))

        merge = lambda *a: jnp.add(*halves(*a))
        r4 = [[merge(part[b][j], part[b][j + 2], 4) for j in range(2)] for b in range(B)]
        r2 = [merge(r4[b][0], r4[b][1], 2) for b in range(B)]
        u, v = halves(r2[0], r2[1], 1)
        o_buf[...] = ((base8 + g8 * u) + g8 * v if FOLD else base8 + g8 * (u + v)).astype(BF16)
        o_copy = pltpu.make_async_copy(o_buf, o_hbm, sem_small.at[0])
        o_copy.start()
        o_copy.wait()

    def fn(A_x, A_c_kv, A_w_q, A_w_uk, A_w_uv, A_w_o, B_x, B_w1, B_b1, B_w2, B_b2):
        hbm = pl.BlockSpec(memory_space=pltpu.HBM)
        dma_sems = pltpu.SemaphoreType.DMA
        w_view, o_view, w1_view, w2_view = (256, 2 * H, D), (8, 32, 16, M), (896, 8, 128), (112, 16, M)
        out = pl.pallas_call(
            _kernel,
            out_shape=jax.ShapeDtypeStruct((8, 128), BF16),
            in_specs=[hbm] * 10,
            out_specs=hbm,
            scratch_shapes=[
                pltpu.VMEM((B, M), BF16), pltpu.VMEM((F,), BF16), pltpu.VMEM((M,), BF16),
                pltpu.VMEM((B, 64, 16, 16, DC), BF16), pltpu.VMEM(w_view, BF16), pltpu.VMEM(w_view, BF16),
                pltpu.VMEM(w_view, BF16), pltpu.VMEM(o_view, BF16),
                pltpu.VMEM(w1_view, BF16), pltpu.VMEM(w2_view, BF16),
                pltpu.VMEM((B, M, 128), F32),
                pltpu.VMEM((DC * 8 + 8, 128), F32),
                pltpu.VMEM((B * H, DC), BF16), pltpu.VMEM((H, DC), F32),
                pltpu.VMEM((H, 128), F32), pltpu.VMEM((H, 128), F32),
                pltpu.VMEM((H, 1024), F32),
                pltpu.VMEM((3 * H, D), F32), pltpu.VMEM((B, 4 * D, 128), F32), pltpu.VMEM((8, 128), F32), pltpu.VMEM((8, 128), BF16),
            ] + ([dma_sems((43 + len(CUTS),))] if ONE else [dma_sems((n,)) for n in (5, 32, 4, len(CUTS) - 1, 3)]),
            compiler_params=pltpu.CompilerParams(
                vmem_limit_bytes=100 * 1024 * 1024, disable_semaphore_checks=True, disable_bounds_checks=True),
        )(A_x.reshape(B, M), A_c_kv.reshape(2048, 16, DC), A_w_q.reshape(w_view), A_w_uk.reshape(w_view),
          A_w_uv.reshape(w_view), A_w_o.reshape(o_view),
          B_w1.reshape(M // 8, 8, F // 128, 128).transpose(0, 2, 1, 3).reshape(w1_view), B_b1,
          B_w2.reshape(w2_view), B_b2)
        return out.reshape(M // 128, B, 128).transpose(1, 0, 2).reshape(B, 1, M)
    return fn


_impl = make(SMALL=1)


@jax.jit
def pallas_recurrent_scan__compressed_kv_cla__dense_activation_gelu__decode_kernel(
    A_x, A_c_kv, A_w_q, A_w_uk, A_w_uv, A_w_o, B_x, B_w1, B_b1, B_w2, B_b2,
):
    return _impl(A_x, A_c_kv, A_w_q, A_w_uk, A_w_uv, A_w_o, B_x, B_w1, B_b1, B_w2, B_b2)
```

```python
import jax
import jax.numpy as jnp
from jax import lax
import jax.experimental.pallas as pl
import jax.experimental.pallas.tpu as pltpu

F32 = jnp.float32
BF16 = jnp.bfloat16

B, H, SK, D, M, DC, F = 2, 32, 16384, 128, 512, 512, 1792
LOG2E = 1.4426950408889634
NT = (((1,), (1,)), ((), ()))

C_VIEW = (B * SK // 16, 16, DC)
W_VIEW = (256, 2 * H, D)
W1_VIEW = (M * F // 1024, 8, 128)
W2_VIEW = (F // 16, 16, M)
O_VIEW = (8, 32, 16, M)


def _runs(name, lo, hi):
    return [(name, run) for run in range(lo, hi)]


PHASES = (
    _runs("uv", 0, 4) + _runs("uk", 0, 4) + _runs("q", 0, 4) + _runs("c", 0, 3) + _runs("w1", 0, 1),
    _runs("c", 3, 16) + _runs("w2", 0, 2) + _runs("w1", 1, 2),
    _runs("c", 16, 32),
)
O_ORDER = (0, 2, 4, 6, 1, 3, 5)
ROUNDS = 3 * 64 + 16
LAG = 2
EDGES = (0, 1, 62, 64, 126, 128, 190, 192, ROUNDS - 2, ROUNDS - 1, ROUNDS)
LAST_CUTS = (0, 8, 16, 20, 24, 26, 28, 30, 31, 32)
BK = 1024
BLOCKS = SK // BK
FIRST, PER_BATCH = 97, 57

SEM_W, SEM_SMALL, SEM_O, SEM_C, SEM_LAST = 0, 5, 8, 12, 12 + B * BLOCKS


def _loop(lo, hi, body):
    lax.fori_loop(lo, hi, lambda i, _: body(i), None)


def _rows8(v):
    return jnp.concatenate([v[:, j * 128:(j + 1) * 128] for j in range(M // 128)], axis=0)


def _kernel(x_hbm, c_hbm, wq_hbm, wuk_hbm, wuv_hbm, wo_hbm, w1_hbm, b1_hbm, w2_hbm, b2_hbm,
            o_hbm,
            x_buf, b1_buf, b2_buf, c_buf, wq_buf, wuk_buf, wuv_buf, wo_buf, w1_buf, w2_buf,
            xs, tmp, qa_ref, s_ref, acc_ref, m_ref, l_ref, ctx_ref, mul_ref, gate_ref, o_buf,
            sems):
    weights = {"q": (wq_hbm, wq_buf, SEM_W), "uk": (wuk_hbm, wuk_buf, SEM_W + 1),
               "uv": (wuv_hbm, wuv_buf, SEM_W + 2), "w1": (w1_hbm, w1_buf, SEM_W + 3),
               "w2": (w2_hbm, w2_buf, SEM_W + 4)}

    def start(src, dst, sem, queue):
        pltpu.make_async_copy(src, dst, sems.at[sem]).start(priority=queue)

    def wait_filled(buf, sem):
        pltpu.make_async_copy(buf, buf, sems.at[sem]).wait()

    def fetch(phase, j, i, queue):
        j = j - 64 * phase
        if phase == len(PHASES):
            if i % 8 < len(O_ORDER):
                at = (O_ORDER[i % 8], 2 * j + i // 8)
                start(wo_hbm.at[at], wo_buf.at[at], SEM_O + (j >> 2), queue)
            return
        name, run = PHASES[phase][i]
        p = 64 * run + j
        if name == "c":
            b = run // 16
            start(c_hbm.at[p], c_buf.at[b, j, run % 16], SEM_C + BLOCKS * b + (j >> 2), queue)
            return
        hbm, buf, sem = weights[name]

        def go():
            at = pl.ds(8 * p, 8) if name == "w1" else p
            start(hbm.at[at], buf.at[at], sem, queue)

        if name in ("w1", "w2") and run == 1:
            pl.when(j < 48)(go)
        else:
            go()

    def fetch_last(p):
        group = max(i for i, cut in enumerate(LAST_CUTS) if cut <= p)
        start(wo_hbm.at[7, p], wo_buf.at[7, p], SEM_LAST + group, 1)

    def issue_round(j, edge):
        on_queue0 = (0, 4, 8, 12) if edge else (None, 6, 8, 12)
        for g in range(4):
            for t in range(3):
                if t == 2 and on_queue0[g] is not None:
                    fetch(edge // 64, j, on_queue0[g], 0)
                if edge + LAG < ROUNDS:
                    fetch((edge + LAG) // 64, j + LAG, 4 * g + 1 + t, 1)
                else:
                    fetch_last(12 * (edge + LAG - ROUNDS) + 3 * g + t)

    def issue(lo, hi, *within):
        for s, e in zip(EDGES, EDGES[1:]):
            if within:
                if any(max(a, s) < min(z, e) for a, z in within):
                    _loop(jnp.clip(lo, s, e), jnp.clip(hi, s, e), lambda j, s=s: issue_round(j, s))
            elif max(lo, s) + 1 == min(hi, e):
                issue_round(max(lo, s), s)
            elif max(lo, s) < min(hi, e):
                _loop(max(lo, s), min(hi, e), lambda j, s=s: issue_round(j, s))

    fill = [(j, i) for j in range(LAG) for i in range(16) if i % 4 and (j, i) not in ((0, 2), (0, 6))]
    for n, (j, i) in enumerate(fill):
        if n in (0, 7, 14):
            fetch(0, 0, 2 * n // 7, 0)
        fetch(0, j, i, 1)
    issue(0, 1)
    x_copy = pltpu.make_async_copy(x_hbm, x_buf, sems.at[SEM_SMALL])
    b1_copy = pltpu.make_async_copy(b1_hbm, b1_buf, sems.at[SEM_SMALL + 1])
    b2_copy = pltpu.make_async_copy(b2_hbm, b2_buf, sems.at[SEM_SMALL + 2])
    for c in (x_copy, b1_copy, b2_copy):
        c.start()
    issue(1, 16)

    x_copy.wait()
    x = x_buf[...].astype(F32)
    xc = x - jnp.mean(x, axis=-1, keepdims=True)
    var = jnp.mean(xc * xc, axis=-1, keepdims=True)
    xn = (xc * lax.rsqrt(var + 1e-5)).astype(BF16)
    xf = xn.astype(F32)
    for b in range(B):
        for j in range(M // 128):
            cols = slice(j * 128, (j + 1) * 128)
            xs[b, cols, :] = jnp.broadcast_to(xf[b:b + 1, cols], (128, 128)).T
    issue(16, 70)

    wait_filled(*weights["q"][1:])

    def q_rows(i, carry):
        q0, q1 = carry
        for u in range(8):
            m = pl.ds(i * 8 + u, 1)
            w = wq_buf[i * 4 + u // 2, pl.ds((u % 2) * H, H)].astype(F32)
            q0 = q0 + xs[0, m, :] * w
            q1 = q1 + xs[1, m, :] * w
        return q0, q1

    def q_step(i, carry):
        issue(70 + 2 * i, 72 + 2 * i, (70, 78))
        return lax.fori_loop(i * 16, i * 16 + 16, q_rows, carry)

    q0, q1 = lax.fori_loop(0, 4, q_step, (jnp.zeros((H, D), F32), jnp.zeros((H, D), F32)))
    q = jnp.concatenate([q0, q1, jnp.zeros((128 - B * H, D), F32)], axis=0).astype(BF16)

    wait_filled(*weights["uk"][1:])
    group = (lax.broadcasted_iota(jnp.int32, (16, 8, 128), 2) % H) // 8

    def qa_step(i):
        issue(78 + 2 * i, 80 + 2 * i, (78, 94))
        for u in range(4):
            w = wuk_buf[pl.ds((i * 4 + u) * 8, 8)].reshape(16 * H, D)
            r = lax.dot_general(w, q, NT, preferred_element_type=F32).reshape(16, 4, 8, 128)
            v = jnp.where(group == 0, r[:, 0],
                          jnp.where(group == 1, r[:, 1], jnp.where(group == 2, r[:, 2], r[:, 3])))
            tmp[pl.ds(pl.multiple_of((i * 4 + u) * 128, 128), 128), :] = v.reshape(128, 128)

    _loop(0, 8, qa_step)
    issue(94, 96)
    sub = lax.broadcasted_iota(jnp.int32, (128, 128), 1) % 8
    for j in range(DC // 128):
        t = tmp[pl.ds(j * 1024, 128, stride=8), :]
        for s in range(1, 8):
            t = jnp.where(sub == s, tmp[pl.ds(j * 1024 + s, 128, stride=8), :], t)
        qa_ref[:, j * 128:(j + 1) * 128] = (t.T[:B * H] * (D ** -0.5 * LOG2E)).astype(BF16)
    wait_filled(*weights["uv"][1:])
    issue(96, FIRST)

    def attend(b):
        def advance(lo, hi, span=None):
            a, z = span or (lo, hi)
            issue(FIRST + PER_BATCH * b + lo, FIRST + PER_BATCH * b + hi,
                  *[(FIRST + PER_BATCH * k + a, FIRST + PER_BATCH * k + z) for k in range(B)])

        heads = pl.ds(pl.multiple_of(b * H, H), H)
        m_ref[...] = jnp.full((H, 128), -jnp.inf, F32)
        l_ref[...] = jnp.zeros((H, 128), F32)
        acc_ref[...] = jnp.zeros((H, DC), F32)

        def keys(i):
            return c_buf[b, pl.ds(i * 4, 4)].reshape(BK, DC)

        def scores(i):
            wait_filled(c_buf.at[b, pl.ds(i * 4, 4)], SEM_C + BLOCKS * b + i)
            return lax.dot_general(qa_ref[heads, :], keys(i), NT, preferred_element_type=F32)

        def accumulate(i):
            sc = s_ref[...]
            m_prev = m_ref[...]
            m_new = jnp.maximum(m_prev, jnp.max(sc, axis=1, keepdims=True))
            p = jnp.exp2(sc - m_new[:, :1])
            alpha = jnp.exp2(m_prev - m_new)
            l_ref[...] = alpha * l_ref[...] + jnp.sum(p, axis=1, keepdims=True)
            m_ref[...] = m_new
            pv = jnp.dot(p.astype(BF16), keys(i), preferred_element_type=F32)
            acc_ref[...] = acc_ref[...] * alpha[:, :1] + pv

        def block(i):
            advance((11 * i) >> 2, (11 * i + 11) >> 2, (2, 44))
            sc = scores(i)
            accumulate(i - 1)
            s_ref[...] = sc

        advance(0, 2)
        s_ref[...] = scores(0)
        _loop(1, BLOCKS, block)
        advance(44, 46)
        accumulate(BLOCKS - 1)

        advance(46, 48)
        pc = acc_ref[...] / l_ref[...][:, :1]
        for j in range(DC // 128):
            cols = slice(j * 128, (j + 1) * 128)
            tmp[cols, :] = jnp.concatenate([pc[:, cols]] * 4, axis=0).T
        quarter = lax.broadcasted_iota(jnp.int32, (128, 128), 1) // H
        flat = tmp[pl.ds(0, 128, stride=4), :]
        for s in range(1, 4):
            flat = jnp.where(quarter == s, tmp[pl.ds(s, 128, stride=4), :], flat)
        tmp[pl.ds(1024, 128), :] = flat
        diag = lax.broadcasted_iota(jnp.int32, (H, 128), 1) % H == lax.broadcasted_iota(jnp.int32, (H, 128), 0)

        def ctx_step(i, ctx):
            advance(48 + 2 * i, 50 + 2 * i, (48, 52))
            a = jnp.concatenate([jnp.where(diag, tmp[pl.ds(1024 + i * 64 + t, 1), :], 0.0) for t in range(64)], axis=1)
            w = wuv_buf[pl.ds(i * 128, 128)].reshape(64 * 128, D)
            return ctx + jnp.dot(a.astype(BF16), w, preferred_element_type=F32)

        ctx_ref[heads, :] = lax.fori_loop(0, 2, ctx_step, jnp.zeros((H, D), F32))

        @pl.when(b == 0)
        def _():
            issue(FIRST + 52, FIRST + 55)
            wait_filled(*weights["w1"][1:])
            b1_copy.wait()
            w1 = jnp.concatenate(
                [jnp.concatenate([w1_buf[r * (F // 128) + j].astype(F32) for r in range(M // 8)], axis=0).astype(BF16)
                 for j in range(F // 128)], axis=1)
            hid = jnp.dot(xn, w1, preferred_element_type=F32)
            hid = jax.nn.gelu(hid + b1_buf[...].astype(F32).reshape(1, F), approximate=True).astype(BF16)
            issue(FIRST + 55, FIRST + PER_BATCH)
            wait_filled(*weights["w2"][1:])
            b2_copy.wait()
            z = jnp.dot(hid, w2_buf[...].reshape(F, M), preferred_element_type=F32)
            z8 = _rows8(z + b2_buf[...].astype(F32).reshape(1, M))
            gate_ref[...] = z8 * jax.nn.sigmoid(z8)

    _loop(0, B, attend)
    issue(FIRST + PER_BATCH + 52, ROUNDS)
    for p in range(12 * LAG, 32):
        fetch_last(p)

    for b in range(B):
        for k in range(4):
            v = ctx_ref[pl.ds(b * H + H - 4 + k, 1), :].astype(BF16).astype(F32)
            mul_ref[b, k * D:(k + 1) * D] = jnp.broadcast_to(v, (128, 128)).T

    def project(k, s):
        wait_filled(wo_buf.at[pl.ds(0, 7), pl.ds(8 * k, 8)], SEM_O + k)
        lhs = jnp.concatenate([ctx_ref[pl.ds(4 * a + k, B, stride=H), :] for a in range(7)], axis=1)
        w = wo_buf[pl.ds(0, 7), pl.ds(8 * k, 8)].reshape(7 * D, M)
        return s + jnp.dot(lhs.astype(BF16), w, preferred_element_type=F32)

    s = lax.fori_loop(0, 4, project, jnp.zeros((B, M), F32))
    g8 = gate_ref[...]
    base8 = _rows8(x) + _rows8(s) * g8

    part = [[None] * (M // 128) for _ in range(B)]
    for i, (lo, hi) in enumerate(zip(LAST_CUTS, LAST_CUTS[1:])):
        wait_filled(wo_buf.at[7, pl.ds(lo, hi - lo)], SEM_LAST + i)
        for r in range(16 * lo, 16 * hi, 8):
            w = wo_buf[7, r // 16, r % 16:r % 16 + 8].astype(F32)
            for b in range(B):
                mul = mul_ref[b, r:r + 8, :]
                for j in range(M // 128):
                    t = w[:, j * 128:(j + 1) * 128] * mul
                    part[b][j] = t if part[b][j] is None else part[b][j] + t

    sl = lax.broadcasted_iota(jnp.int32, (8, 128), 0)

    def merge(lo, hi, k):
        m = (sl & k) != 0
        if k == 4:
            return jnp.where(m, hi, lo) + pltpu.roll(jnp.where(m, lo, hi), 4, 0)
        return jnp.where(m, hi, lo) + jnp.where(m, pltpu.roll(hi, k, 0), pltpu.roll(lo, 8 - k, 0))

    r4 = [[merge(part[b][j], part[b][j + 2], 4) for j in range(2)] for b in range(B)]
    r2 = [merge(r4[b][0], r4[b][1], 2) for b in range(B)]
    o_buf[...] = (base8 + g8 * merge(r2[0], r2[1], 1)).astype(BF16)
    o_copy = pltpu.make_async_copy(o_buf, o_hbm, sems.at[SEM_SMALL])
    o_copy.start()
    o_copy.wait()


@jax.jit
def pallas_recurrent_scan__compressed_kv_cla__dense_activation_gelu__decode_kernel(
    A_x: jax.Array,
    A_c_kv: jax.Array,
    A_w_q: jax.Array,
    A_w_uk: jax.Array,
    A_w_uv: jax.Array,
    A_w_o: jax.Array,
    B_x: jax.Array,
    B_w1: jax.Array,
    B_b1: jax.Array,
    B_w2: jax.Array,
    B_b2: jax.Array,
):
    del B_x
    hbm = pl.BlockSpec(memory_space=pltpu.HBM)
    w1_tiles = B_w1.reshape(M // 8, 8, F // 128, 128).transpose(0, 2, 1, 3).reshape(W1_VIEW)
    out = pl.pallas_call(
        _kernel,
        out_shape=jax.ShapeDtypeStruct((8, 128), BF16),
        in_specs=[hbm] * 10,
        out_specs=hbm,
        scratch_shapes=[
            pltpu.VMEM((B, M), BF16), pltpu.VMEM((F,), BF16), pltpu.VMEM((M,), BF16),
            pltpu.VMEM((B, 64, 16, 16, DC), BF16),
            pltpu.VMEM(W_VIEW, BF16), pltpu.VMEM(W_VIEW, BF16), pltpu.VMEM(W_VIEW, BF16),
            pltpu.VMEM(O_VIEW, BF16), pltpu.VMEM(W1_VIEW, BF16), pltpu.VMEM(W2_VIEW, BF16),
            pltpu.VMEM((B, M, 128), F32), pltpu.VMEM((DC * 8 + 8, 128), F32),
            pltpu.VMEM((B * H, DC), BF16), pltpu.VMEM((H, BK), F32), pltpu.VMEM((H, DC), F32),
            pltpu.VMEM((H, 128), F32), pltpu.VMEM((H, 128), F32),
            pltpu.VMEM((3 * H, D), F32), pltpu.VMEM((B, 4 * D, 128), F32),
            pltpu.VMEM((8, 128), F32), pltpu.VMEM((8, 128), BF16),
            pltpu.SemaphoreType.DMA((SEM_LAST + len(LAST_CUTS) - 1,)),
        ],
        compiler_params=pltpu.CompilerParams(
            vmem_limit_bytes=100 * 1024 * 1024, disable_semaphore_checks=True, disable_bounds_checks=True),
    )(A_x.reshape(B, M), A_c_kv.reshape(C_VIEW), A_w_q.reshape(W_VIEW), A_w_uk.reshape(W_VIEW),
      A_w_uv.reshape(W_VIEW), A_w_o.reshape(O_VIEW), w1_tiles, B_b1, B_w2.reshape(W2_VIEW), B_b2)
    return out.reshape(M // 128, B, 128).transpose(1, 0, 2).reshape(B, 1, M)
```
